```python
import jax
import jax.numpy as jnp

def _softmax(x, axis=-1):
    return jax.nn.softmax(x, axis=axis)
def _gelu(x):
    return jax.nn.gelu(x, approximate=True)
def _silu(x):
    return jax.nn.silu(x)
def _sigmoid(x):
    return jax.nn.sigmoid(x)
def _layernorm(x, axis=-1, eps=1e-5):
    m = jnp.mean(x, axis=axis, keepdims=True)
    v = jnp.var(x, axis=axis, keepdims=True)
    return (x - m) / jnp.sqrt(v + eps)
def _scatter_add(tgt, idx, src, axis=0):
    return tgt.at[idx].add(src)
def _segment_sum(src, seg, n):
    return jax.ops.segment_sum(src, seg, n)
class _Rng:
    def __init__(self, key):
        self._k = key
    def _next(self):
        self._k, sub = jax.random.split(self._k)
        return sub
    def normal(self, shape):
        return jax.random.normal(self._next(), shape, dtype=jnp.bfloat16)
    def randint(self, lo, hi, shape):
        return jax.random.randint(self._next(), shape, lo, hi, dtype=jnp.int32)
    def uniform(self, shape, lo=0.0, hi=1.0):
        return jax.random.uniform(self._next(), shape, jnp.bfloat16, lo, hi)
    def permutation(self, n):
        return jax.random.permutation(self._next(), n)


kernel_name = 'recurrent_scan__sliding_local_dilated__glu_gated_swiglu__prompt'

def setup_inputs():
    _rng = _Rng(jax.random.key(int.from_bytes(__import__("os").urandom(4), "little")))
    _w = (lambda a: (lambda t: t.astype(jnp.bfloat16) if jnp.issubdtype(t.dtype, jnp.floating) else t)(jnp.asarray(a)))
    def _A_setup():
        B, S, D = 1, 2048, 1024
        return {
            "x": _w((lambda *s: _rng.normal(s) * 0.05)(B, S, D)),
            "wqkv": _w((lambda *s: _rng.normal(s) * 0.05)(D, 3 * D)),
            "wo": _w((lambda *s: _rng.normal(s) * 0.05)(D, D)),
        }
    _A_in = _A_setup()

    def _B_setup():
        B, S, D, F = 1, 2048, 1024, 3584
        return {
            "x": _w((lambda *s: _rng.normal(s) * 0.05)(B, S, D)),
            "w1": _w((lambda *s: _rng.normal(s) * 0.05)(D, F) * (2.0 / D) ** 0.5),
            "w3": _w((lambda *s: _rng.normal(s) * 0.05)(D, F) * (2.0 / D) ** 0.5),
            "w2": _w((lambda *s: _rng.normal(s) * 0.05)(F, D) * (2.0 / F) ** 0.5),
        }
    _B_in = _B_setup()

    return {
        "A_x": _A_in["x"],
        "A_wqkv": _A_in["wqkv"],
        "A_wo": _A_in["wo"],
        "B_x": _B_in["x"],
        "B_w1": _B_in["w1"],
        "B_w3": _B_in["w3"],
        "B_w2": _B_in["w2"],
    }

def reference(A_x, A_wqkv, A_wo, B_x, B_w1, B_w3, B_w2):
    def _A_ref(x, wqkv, wo):
        B, S, D = x.shape
        H = 32; Dh = D // H
        W, dil = 8, 2
        qkv = (lambda x, *d: x.transpose(*d))((x @ wqkv).reshape(B, S, 3, H, Dh), 2, 0, 3, 1, 4)
        q, k, v = qkv[0], qkv[1], qkv[2]
        scale = Dh ** -0.5
        pos = jnp.arange(S)
        off = jnp.arange(W) * dil
        idx = pos[:, None] - off[None, :]
        mask = idx >= 0
        idx_c = jnp.where(mask, idx, 0).reshape(-1)
        kg = k[:, :, idx_c, :].reshape(B, H, S, W, Dh)
        vg = v[:, :, idx_c, :].reshape(B, H, S, W, Dh)
        logits = jnp.einsum("bhsd,bhswd->bhsw", q, kg) * scale
        logits = jnp.where(mask[None, None, :, :], logits, -1e9)
        attn = _softmax(logits, axis=-1)
        o = jnp.einsum("bhsw,bhswd->bhsd", attn, vg)
        return (lambda x, *d: x.transpose(*d))(o, 0, 2, 1, 3).reshape(B, S, D) @ wo

    def _B_ref(x, w1, w3, w2):
        gate = jnp.einsum("bsd,df->bsf", x, w1)
        up = jnp.einsum("bsd,df->bsf", x, w3)
        h = _silu(gate) * up
        out = jnp.einsum("bsf,fd->bsd", h, w2)
        return out

    x = A_x
    xn = _layernorm(x, axis=-1)
    s = _A_ref(xn, A_wqkv, A_wo)
    g = _silu(_B_ref(xn, B_w1, B_w3, B_w2))
    return x + s * g
```

```python
import jax
import jax.numpy as jnp
from jax import lax
import jax.experimental.pallas as pl
import jax.experimental.pallas.tpu as pltpu

S, D, H, DH, F, W, DIL = 2048, 1024, 32, 32, 3584, 8, 2
HALO = 16
PS = 33
NT = (((1,), (1,)), ((), ()))


def silu(g):
    t = 0.5 * g
    return t + t * jnp.tanh(t)


def _make_kernel(tm=256, fc=512, ar=16, groups=((0, 1), (2, 3), (4, 5), (6,)), skip_main=False):
    nsteps = S // tm
    nch = F // fc
    ng = len(groups)
    grp_of = {c: gi for gi, g in enumerate(groups) for c in g}

    def kernel(x_ref, wqkv_hbm, wo_hbm, w1_hbm, w3_hbm, w2_hbm, o_ref,
               wqkv_ref, wo_ref, w1_ref, w3_ref, w2_ref,
               wt_ref, wop_ref, t_ref, q_ref, k_ref, v_ref, sems):
        i = pl.program_id(0)

        def cp_qkv(sec):
            return pltpu.make_async_copy(wqkv_hbm.at[:, sec * D:(sec + 1) * D], wqkv_ref.at[sec], sems.at[sec])

        def cp_wo():
            return pltpu.make_async_copy(wo_hbm, wo_ref, sems.at[3])

        def cp_ffn(gi):
            c0, c1 = groups[gi][0] * fc, (groups[gi][-1] + 1) * fc
            return [
                pltpu.make_async_copy(w1_hbm.at[:, c0:c1], w1_ref.at[:, c0:c1], sems.at[4 + 3 * gi]),
                pltpu.make_async_copy(w3_hbm.at[:, c0:c1], w3_ref.at[:, c0:c1], sems.at[5 + 3 * gi]),
                pltpu.make_async_copy(w2_hbm.at[c0:c1, :], w2_ref.at[c0:c1, :], sems.at[6 + 3 * gi]),
            ]

        @pl.when(i == 0)
        def _prep():
            for sec in range(3):
                cp_qkv(sec).start()
            cp_wo().start()
            for gi in range(ng):
                for c in cp_ffn(gi):
                    c.start()
            eye = (lax.broadcasted_iota(jnp.int32, (128, 128), 0)
                   == lax.broadcasted_iota(jnp.int32, (128, 128), 1)).astype(jnp.bfloat16)

            def sec_body(sec):
                def body(cb, _):
                    c0 = pl.multiple_of(cb * 128, 128)
                    tt = lax.dot_general(eye, wqkv_ref[sec, :, pl.ds(c0, 128)], NT,
                                         preferred_element_type=jnp.float32)
                    for hl in range(4):
                        for kb in range(8):
                            t_ref[kb, pl.ds((cb * 4 + hl) * PS, DH), :] = (
                                tt[hl * DH:(hl + 1) * DH, kb * 128:(kb + 1) * 128])
                    return 0
                lax.fori_loop(0, 8, body, 0)

                def body2(dd, _):
                    for dl in range(4):
                        d = dd * 4 + dl
                        r0 = pl.multiple_of(sec * D + d * H, H)
                        for kb in range(8):
                            wt_ref[kb, pl.ds(r0, H), :] = (
                                t_ref[kb, pl.ds(d, H, stride=PS), :].astype(jnp.bfloat16))
                    return 0
                lax.fori_loop(0, DH // 4, body2, 0)

            for sec in range(3):
                cp_qkv(sec).wait()
                sec_body(sec)
            cp_wo().wait()

            def body3a(hh, _):
                for hl in range(4):
                    h = hh * 4 + hl
                    blk = wo_ref[pl.ds(pl.multiple_of(h * DH, DH), DH), :].astype(jnp.float32)
                    for j in range(8):
                        t_ref[j, pl.ds(h * PS, DH), :] = blk[:, j * 128:(j + 1) * 128]
                return 0
            lax.fori_loop(0, H // 4, body3a, 0)

            def body3(dd, _):
                for dl in range(4):
                    d = dd * 4 + dl
                    r0 = pl.multiple_of(d * H, H)
                    for j in range(8):
                        wop_ref[j, pl.ds(r0, H), :] = (
                            t_ref[j, pl.ds(d, H, stride=PS), :].astype(jnp.bfloat16))
                return 0
            lax.fori_loop(0, DH // 4, body3, 0)
            k_ref[:, 0:HALO, :] = jnp.zeros((8, HALO, 128), jnp.float32)
            v_ref[:, 0:HALO, :] = jnp.zeros((8, HALO, 128), jnp.float32)
            if skip_main:
                for gi in range(ng):
                    for c in cp_ffn(gi):
                        c.wait()

        if skip_main:
            o_ref[...] = x_ref[...]
            return

        x = x_ref[...].astype(jnp.float32)
        mu = jnp.mean(x, axis=-1, keepdims=True)
        xc = x - mu
        var = jnp.mean(xc * xc, axis=-1, keepdims=True)
        xn = (xc * lax.rsqrt(var + 1e-5)).astype(jnp.bfloat16)

        def wt_block(cb):
            return jnp.concatenate([wt_ref[kb, cb * 128:(cb + 1) * 128, :] for kb in range(8)], axis=1)

        for j in range(8):
            q_ref[j] = lax.dot_general(xn, wt_block(j), NT, preferred_element_type=jnp.float32)
        for j in range(8):
            k_ref[j, HALO:, :] = lax.dot_general(xn, wt_block(8 + j), NT, preferred_element_type=jnp.float32)
        for j in range(8):
            v_ref[j, HALO:, :] = lax.dot_general(xn, wt_block(16 + j), NT, preferred_element_type=jnp.float32)

        def ffn_chunk(c, acc):
            if groups[grp_of[c]][0] == c:
                @pl.when(i == 0)
                def _():
                    for cp in cp_ffn(grp_of[c]):
                        cp.wait()
            g = jnp.dot(xn, w1_ref[:, c * fc:(c + 1) * fc], preferred_element_type=jnp.float32)
            u = jnp.dot(xn, w3_ref[:, c * fc:(c + 1) * fc], preferred_element_type=jnp.float32)
            h = (silu(g) * u).astype(jnp.bfloat16)
            t = jnp.dot(h, w2_ref[c * fc:(c + 1) * fc, :], preferred_element_type=jnp.float32)
            return t if acc is None else acc + t

        acc = ffn_chunk(0, None)

        scale = DH ** -0.5
        a_rows = []
        for r in range(tm // ar):
            r0 = r * ar
            qs = [q_ref[j, r0:r0 + ar, :] for j in range(8)]
            pos = i * tm + r0 + lax.broadcasted_iota(jnp.int32, (ar, 128), 0)
            logits = []
            for w in range(W):
                b = HALO + r0 - DIL * w
                s = qs[0] * k_ref[0, b:b + ar, :]
                for j in range(1, 8):
                    s = s + qs[j] * k_ref[j, b:b + ar, :]
                s = s + pltpu.roll(s, 64, 1)
                s = s + pltpu.roll(s, 32, 1)
                s = s * scale
                if r0 < DIL * w:
                    s = jnp.where(pos >= DIL * w, s, -1e9)
                logits.append(s)
            m = logits[0]
            for w in range(1, W):
                m = jnp.maximum(m, logits[w])
            es = [jnp.exp(l - m) for l in logits]
            den = es[0]
            for w in range(1, W):
                den = den + es[w]
            inv = 1.0 / den
            ps = [e * inv for e in es]
            outs = []
            for j in range(8):
                acc_a = None
                for w in range(W):
                    b = HALO + r0 - DIL * w
                    t = ps[w] * v_ref[j, b:b + ar, :]
                    acc_a = t if acc_a is None else acc_a + t
                outs.append(acc_a.astype(jnp.bfloat16))
            a_rows.append(jnp.concatenate(outs, axis=1))
        a = jnp.concatenate(a_rows, axis=0)

        k_ref[:, 0:HALO, :] = k_ref[:, tm:tm + HALO, :]
        v_ref[:, 0:HALO, :] = v_ref[:, tm:tm + HALO, :]

        for c in range(1, nch - 1):
            acc = ffn_chunk(c, acc)
        wop = jnp.concatenate([wop_ref[j] for j in range(8)], axis=1)
        s_out = jnp.dot(a, wop, preferred_element_type=jnp.float32)
        acc = ffn_chunk(nch - 1, acc)
        o_ref[...] = (x + s_out * silu(acc)).astype(o_ref.dtype)

    def fn(A_x, A_wqkv, A_wo, B_x, B_w1, B_w3, B_w2):
        x = A_x.reshape(S, D)
        anyspec = pl.BlockSpec(memory_space=pl.ANY)
        out = pl.pallas_call(
            kernel,
            grid=(nsteps,),
            in_specs=[pl.BlockSpec((tm, D), lambda i: (i, 0))] + [anyspec] * 5,
            out_specs=pl.BlockSpec((tm, D), lambda i: (i, 0)),
            out_shape=jax.ShapeDtypeStruct((S, D), jnp.bfloat16),
            scratch_shapes=[
                pltpu.VMEM((3, D, D), jnp.bfloat16),
                pltpu.VMEM((D, D), jnp.bfloat16),
                pltpu.VMEM((D, F), jnp.bfloat16),
                pltpu.VMEM((D, F), jnp.bfloat16),
                pltpu.VMEM((F, D), jnp.bfloat16),
                pltpu.VMEM((8, 3 * D, 128), jnp.bfloat16),
                pltpu.VMEM((8, D, 128), jnp.bfloat16),
                pltpu.VMEM((8, H * PS, 128), jnp.float32),
                pltpu.VMEM((8, tm, 128), jnp.float32),
                pltpu.VMEM((8, tm + HALO, 128), jnp.float32),
                pltpu.VMEM((8, tm + HALO, 128), jnp.float32),
                pltpu.SemaphoreType.DMA((4 + 3 * ng,)),
            ],
            compiler_params=pltpu.CompilerParams(
                dimension_semantics=("arbitrary",), vmem_limit_bytes=110 * 1024 * 1024),
        )(x, A_wqkv, A_wo, B_w1, B_w3, B_w2)
        return out.reshape(1, S, D)

    return fn


_fn = _make_kernel()


@jax.jit
def pallas_recurrent_scan__sliding_local_dilated__glu_gated_swiglu__prompt_kernel(
    A_x: jax.Array,
    A_wqkv: jax.Array,
    A_wo: jax.Array,
    B_x: jax.Array,
    B_w1: jax.Array,
    B_w3: jax.Array,
    B_w2: jax.Array,
):
    return _fn(A_x, A_wqkv, A_wo, B_x, B_w1, B_w3, B_w2)
```

```python
import contextlib
import jax
import jax.numpy as jnp
from jax import lax
import jax.experimental.pallas as pl
import jax.experimental.pallas.tpu as pltpu

S, D, H, DH, F, W, DIL = 2048, 1024, 32, 32, 3584, 8, 2
HALO = 16
PS = 33
NT = (((1,), (1,)), ((), ()))
NB = D // 128


def zero_dep(x):
    return jnp.where(x > jnp.inf, 1.0, 0.0).astype(jnp.float32)


def silu(g):
    t = 0.5 * g
    return t + t * jnp.tanh(t)


def layernorm_bf16(x, dep=None):
    x = x.astype(jnp.float32)
    sm = jnp.sum(x, axis=-1, keepdims=True)
    if dep is not None:
        sm = sm + dep
    mu = sm * (1.0 / D)
    xc = x - mu
    var = jnp.mean(xc * xc, axis=-1, keepdims=True)
    rstd = lax.rsqrt(var + 1e-5)
    return (xc * rstd).astype(jnp.bfloat16), zero_dep(rstd)


def pack(x):
    return pltpu.bitcast(x, jnp.uint32)


def unpack(x):
    return pltpu.bitcast(x, jnp.bfloat16)


def _make_kernel(tm=256, fc=512, ar=8, skew=4, attn_pos=1, wo_pos=6, scopes=False, lr=8, bar_pos=None, attn_in_a=False, chain=2, ln_chain=True, xa_copy=True, wo_chain=True, xlu_blocks=(0, 1), safe_dep=True):
    nblk = S // tm
    nch = F // fc
    scope = jax.named_scope if scopes else (lambda n: contextlib.nullcontext())
    SWO, SW1, SW3, SW2, SX = 3, 4, 5, 6, 7

    def kernel(x_hbm, wqkv_hbm, wo_hbm, w1_hbm, w3_hbm, w2_hbm, o_ref,
               wqkv_ref, wo_ref, w1_ref, w3_ref, w2_ref,
               wt_ref, wop_ref, wc_ref, t_ref, t2_ref, x_ref, xn_ref, xa_ref, qkv_ref, sems):
        s = pl.program_id(0)

        def cp_sec(sec):
            if isinstance(sec, int):
                sl = slice(sec * D, (sec + 1) * D)
            else:
                sl = pl.ds(pl.multiple_of(sec * D, D), D)
            return pltpu.make_async_copy(wqkv_hbm.at[:, sl], wqkv_ref.at[:, sl], sems.at[sec])
        cp_wo = lambda: pltpu.make_async_copy(wo_hbm, wo_ref, sems.at[SWO])
        cp_w1 = lambda: pltpu.make_async_copy(w1_hbm, w1_ref, sems.at[SW1])
        cp_w3 = lambda: pltpu.make_async_copy(w3_hbm, w3_ref, sems.at[SW3])
        cp_w2 = lambda: pltpu.make_async_copy(w2_hbm, w2_ref, sems.at[SW2])

        def cp_x(blk):
            if isinstance(blk, int):
                src = x_hbm.at[blk * tm:(blk + 1) * tm, :]
            else:
                src = x_hbm.at[pl.ds(pl.multiple_of(blk * tm, tm), tm), :]
            return pltpu.make_async_copy(src, x_ref.at[blk], sems.at[SX + blk])

        def do_ln(dst_blk, src_blk):
            dep = None
            for r0 in range(0, tm, lr):
                xn, d2 = layernorm_bf16(x_ref[src_blk, r0:r0 + lr, :], dep)
                dep = d2 if ln_chain else None
                for kb in range(NB):
                    xn_ref[dst_blk, kb, r0 // 2:(r0 + lr) // 2, :] = pack(xn[:, kb * 128:(kb + 1) * 128])

        def load_xn(blk):
            return jnp.concatenate([unpack(xn_ref[blk, kb]) for kb in range(NB)], axis=1)

        def wt_block(cb):
            return jnp.concatenate([unpack(wt_ref[kb, cb * 64:(cb + 1) * 64, :]) for kb in range(NB)], axis=1)

        def load_xa():
            return jnp.concatenate([unpack(xa_ref[kb]) for kb in range(NB)], axis=1)

        def proj(sec, off, blk, wblock):
            for j in range(NB):
                qkv_ref[sec, j, pl.ds(off, tm), :] = lax.dot_general(
                    load_xa() if blk is None else load_xn(blk), wblock(j), NT, preferred_element_type=jnp.float32)

        def prep_wo_cols(j0, ncols):
            dep = None
            for jj in range(ncols):
                c0 = pl.multiple_of((j0 + jj) * 128, 128)
                for h in range(H):
                    blk = wo_ref[h * DH:(h + 1) * DH, pl.ds(c0, 128)].astype(jnp.float32)
                    if dep is not None:
                        blk = blk + dep
                    if wo_chain:
                        dep = zero_dep(blk[0:1, :])
                    t2_ref[jj, h * PS:h * PS + DH, :] = blk
                for d in range(DH):
                    blk = t2_ref[jj, pl.ds(d, H, stride=PS), :]
                    if dep is not None:
                        blk = blk + dep
                    if wo_chain:
                        dep = zero_dep(blk[0:1, :])
                    wop_ref[j0 + jj, d * (H // 2):(d + 1) * (H // 2), :] = pack(blk.astype(jnp.bfloat16))

        @pl.when(s == 0)
        def _prologue():
            for cp in (cp_x(0), cp_sec(0), cp_sec(1), cp_x(1), cp_sec(2), cp_wo(), cp_x(2), cp_x(3),
                       cp_w1(), cp_x(4), cp_w3(), cp_x(5), cp_x(6), cp_w2(), cp_x(7)):
                cp.start()
            qkv_ref[1:3, :, 0:HALO, :] = jnp.zeros((2, NB, HALO, 128), jnp.float32)
            eye = (lax.broadcasted_iota(jnp.int32, (128, 128), 0)
                   == lax.broadcasted_iota(jnp.int32, (128, 128), 1)).astype(jnp.bfloat16)

            def ln_loop(blk):
                cp_x(blk).wait()

                def body(t, _):
                    for u in range(4):
                        r0 = pl.multiple_of(t * 64 + u * 16, 16)
                        xn, _ = layernorm_bf16(x_ref[blk, pl.ds(r0, 16), :])
                        for kb in range(NB):
                            xn_ref[blk, kb, pl.ds(pl.multiple_of(t * 32 + u * 8, 8), 8), :] = pack(xn[:, kb * 128:(kb + 1) * 128])
                    return 0
                lax.fori_loop(0, tm // 64, body, 0)

            with scope("p_ln0"):
                ln_loop(0)
                for kb in range(NB):
                    xa_ref[kb] = xn_ref[0, kb]

            def sec_body(sec, _):
                cp_sec(sec).wait()

                @pl.when(sec == 1)
                def _():
                    cp_x(1).wait()
                for cb in range(NB):
                    c0 = pl.multiple_of(sec * D + cb * 128, 128)
                    if cb in xlu_blocks:
                        tt = wqkv_ref[:, pl.ds(c0, 128)].astype(jnp.float32).T
                    else:
                        tt = lax.dot_general(eye, wqkv_ref[:, pl.ds(c0, 128)], NT, preferred_element_type=jnp.float32)
                    for hl in range(4):
                        r0 = (cb * 4 + hl) * PS
                        for kb in range(NB):
                            t_ref[kb, r0:r0 + DH, :] = tt[hl * DH:(hl + 1) * DH, kb * 128:(kb + 1) * 128]
                for d in range(DH):
                    r0 = d * (H // 2)
                    rd = pl.multiple_of(sec * (D // 2) + r0, H // 2)
                    for kb in range(NB):
                        blk = pack(t_ref[kb, pl.ds(d, H, stride=PS), :].astype(jnp.bfloat16))
                        wc_ref[kb, r0:r0 + H // 2, :] = blk
                        wt_ref[kb, pl.ds(rd, H // 2), :] = blk
                proj(sec, HALO, None, lambda j: jnp.concatenate(
                    [unpack(wc_ref[kb, j * 64:(j + 1) * 64, :]) for kb in range(NB)], axis=1))
                do_ln(jnp.where(sec == 0, nblk, 1), jnp.minimum(sec, 1))
                return 0

            with scope("p_sec"):
                lax.fori_loop(0, 3, sec_body, 0)

        @pl.when(jnp.logical_and(s > 0, s < nblk))
        def _seg_a():
          with scope("segA"):
            @pl.when(s < nblk - 1)
            def _():
                cp_x(s + 1).wait()

            @pl.when(s == 1)
            def _():
                cp_wo().wait()
            row0 = pl.multiple_of(s * tm, tm)
            if xa_copy:
                for kb in range(NB):
                    xa_ref[kb] = xn_ref[s, kb]
            for sec in range(3):
                proj(sec, HALO + row0, None if xa_copy else s, lambda j, sec=sec: wt_block(sec * NB + j))
            do_ln(s + 1, jnp.minimum(s + 1, nblk - 1))
            prep_wo_cols(((s - 1) * 2) % NB, 2)

        @pl.when(s >= skew)
        def _seg_bc():
          with scope("segBC"):
            b = s - skew
            row0 = pl.multiple_of(b * tm, tm)

            @pl.when(s == skew)
            def _():
                cp_w1().wait()
                cp_w3().wait()
                cp_w2().wait()

            def ffn_chunk(c, acc):
                sl = slice(c * fc, (c + 1) * fc)
                g = jnp.dot(load_xn(b), w1_ref[:, sl], preferred_element_type=jnp.float32)
                u = jnp.dot(load_xn(b), w3_ref[:, sl], preferred_element_type=jnp.float32)
                h = (silu(g) * u).astype(jnp.bfloat16)
                t = jnp.dot(h, w2_ref[sl, :], preferred_element_type=jnp.float32)
                return t if acc is None else acc + t

            def attention():
                scale = DH ** -0.5
                a_rows = []
                dep = None
                for r in range(tm // ar):
                    r0 = r * ar
                    qs = [qkv_ref[0, j, pl.ds(row0 + (HALO + r0), ar), :] for j in range(NB)]
                    if dep is not None:
                        if chain == 3:
                            qs = [q + dep for q in qs]
                        else:
                            qs[0] = qs[0] + dep
                    logits = []
                    for w in range(W):
                        base = row0 + (HALO + r0 - DIL * w)
                        sc = qs[0] * qkv_ref[1, 0, pl.ds(base, ar), :]
                        for j in range(1, NB):
                            sc = sc + qs[j] * qkv_ref[1, j, pl.ds(base, ar), :]
                        sc = sc + pltpu.roll(sc, 64, 1)
                        sc = sc + pltpu.roll(sc, 32, 1)
                        sc = sc * scale
                        if r0 < DIL * w:
                            pos = row0 + r0 + lax.broadcasted_iota(jnp.int32, (ar, 128), 0)
                            sc = jnp.where(pos >= DIL * w, sc, -1e9)
                        logits.append(sc)
                    m = logits[0]
                    for w in range(1, W):
                        m = jnp.maximum(m, logits[w])
                    es = [jnp.exp(l - m) for l in logits]
                    den = es[0]
                    for w in range(1, W):
                        den = den + es[w]
                    inv = 1.0 / den
                    if chain in (1, 3):
                        dep = zero_dep(inv)
                    ps = [e * inv for e in es]
                    outs = []
                    for j in range(NB):
                        acc_a = None
                        for w in range(W):
                            base = row0 + (HALO + r0 - DIL * w)
                            t = ps[w] * qkv_ref[2, j, pl.ds(base, ar), :]
                            acc_a = t if acc_a is None else acc_a + t
                        outs.append(acc_a)
                    if chain == 2:
                        dep = zero_dep(outs[-1])
                    a_rows.append(jnp.concatenate(outs, axis=1))
                return jnp.concatenate(a_rows, axis=0).astype(jnp.bfloat16)

            acc = None
            a = None
            s_out = None
            for c in range(nch):
                if c == attn_pos:
                    a = attention()
                if c == wo_pos:
                    wop = jnp.concatenate([unpack(wop_ref[j]) for j in range(NB)], axis=1)
                    s_out = jnp.dot(a, wop, preferred_element_type=jnp.float32)
                acc = ffn_chunk(c, acc)
            if wo_pos >= nch:
                wop = jnp.concatenate([unpack(wop_ref[j]) for j in range(NB)], axis=1)
                s_out = jnp.dot(a, wop, preferred_element_type=jnp.float32)
            o_ref[...] = (x_ref[b].astype(jnp.float32) + s_out * silu(acc)).astype(o_ref.dtype)

    def fn(A_x, A_wqkv, A_wo, B_x, B_w1, B_w3, B_w2):
        x = A_x.reshape(S, D)
        anyspec = pl.BlockSpec(memory_space=pl.ANY)
        out = pl.pallas_call(
            kernel,
            grid=(nblk + skew,),
            in_specs=[anyspec] * 6,
            out_specs=pl.BlockSpec((tm, D), lambda s: (jnp.maximum(s - skew, 0), 0)),
            out_shape=jax.ShapeDtypeStruct((S, D), jnp.bfloat16),
            scratch_shapes=[
                pltpu.VMEM((D, 3 * D), jnp.bfloat16),
                pltpu.VMEM((D, D), jnp.bfloat16),
                pltpu.VMEM((D, F), jnp.bfloat16),
                pltpu.VMEM((D, F), jnp.bfloat16),
                pltpu.VMEM((F, D), jnp.bfloat16),
                pltpu.VMEM((NB, 3 * D // 2, 128), jnp.uint32),
                pltpu.VMEM((NB, D // 2, 128), jnp.uint32),
                pltpu.VMEM((NB, D // 2, 128), jnp.uint32),
                pltpu.VMEM((NB, H * PS, 128), jnp.float32),
                pltpu.VMEM((2, H * PS, 128), jnp.float32),
                pltpu.VMEM((nblk, tm, D), jnp.bfloat16),
                pltpu.VMEM((nblk + 1, NB, tm // 2, 128), jnp.uint32),
                pltpu.VMEM((NB, tm // 2, 128), jnp.uint32),
                pltpu.VMEM((3, NB, S + HALO, 128), jnp.float32),
                pltpu.SemaphoreType.DMA((SX + nblk,)),
            ],
            compiler_params=pltpu.CompilerParams(
                dimension_semantics=("arbitrary",), vmem_limit_bytes=120 * 1024 * 1024),
        )(x, A_wqkv, A_wo, B_w1, B_w3, B_w2)
        return out.reshape(1, S, D)

    return fn


_fn = _make_kernel()


@jax.jit
def pallas_recurrent_scan__sliding_local_dilated__glu_gated_swiglu__prompt_kernel(
    A_x: jax.Array,
    A_wqkv: jax.Array,
    A_wo: jax.Array,
    B_x: jax.Array,
    B_w1: jax.Array,
    B_w3: jax.Array,
    B_w2: jax.Array,
):
    return _fn(A_x, A_wqkv, A_wo, B_x, B_w1, B_w3, B_w2)
```

```python
import contextlib
import jax
import jax.numpy as jnp
from jax import lax
import jax.experimental.pallas as pl
import jax.experimental.pallas.tpu as pltpu

S, D, H, DH, F, W, DIL = 2048, 1024, 32, 32, 3584, 8, 2
HALO = 16
PS = 33
NT = (((1,), (1,)), ((), ()))
NB = D // 128


def zero_dep(x):
    return jnp.where(x > jnp.inf, 1.0, 0.0).astype(jnp.float32)


def silu(g):
    t = 0.5 * g
    return t + t * jnp.tanh(t)


def layernorm_bf16(x, dep=None):
    x = x.astype(jnp.float32)
    sm = jnp.sum(x, axis=-1, keepdims=True)
    if dep is not None:
        sm = sm + dep
    mu = sm * (1.0 / D)
    xc = x - mu
    var = jnp.mean(xc * xc, axis=-1, keepdims=True)
    rstd = lax.rsqrt(var + 1e-5)
    return (xc * rstd).astype(jnp.bfloat16), zero_dep(rstd)


def pack(x):
    return pltpu.bitcast(x, jnp.uint32)


def unpack(x):
    return pltpu.bitcast(x, jnp.bfloat16)


def _make_kernel(tm=256, fc=512, ar=8, skew=3, attn_pos=1, wo_pos=7, scopes=False, lr=8,
                xlu_blocks=(0, 1), x_chain=False, p_rows=16, p_chains=1, xlu2=(0, 1, 2, 3, 4, 5, 6, 7)):
    nblk = S // tm
    nch = F // fc
    scope = jax.named_scope if scopes else (lambda n: contextlib.nullcontext())
    SQB, SWO, SW1, SW3, SW2, SX = 3, 4, 5, 6, 7, 8

    def kernel(x_hbm, wqkv_hbm, wo_hbm, w1_hbm, w3_hbm, w2_hbm, o_ref,
               wqkv_ref, wo_ref, w1_ref, w3_ref, w2_ref,
               wt_ref, wop_ref, wc_ref, t_ref, t2_ref, x_ref, xn_ref, xa_ref, xa1_ref, qkv_ref, sems):
        s = pl.program_id(0)

        def cp_cols(c0, n, sem):
            sl = slice(c0, c0 + n) if isinstance(c0, int) else pl.ds(pl.multiple_of(c0, D), n)
            return pltpu.make_async_copy(wqkv_hbm.at[:, sl], wqkv_ref.at[:, sl], sems.at[sem])

        cp_qa = lambda: cp_cols(0, D // 2, 0)
        cp_qb = lambda: cp_cols(D // 2, D // 2, SQB)
        cp_sec = lambda sec: cp_cols(sec * D, D, sec)
        cp_wo = lambda: pltpu.make_async_copy(wo_hbm, wo_ref, sems.at[SWO])
        cp_w1 = lambda: pltpu.make_async_copy(w1_hbm, w1_ref, sems.at[SW1])
        cp_w3 = lambda: pltpu.make_async_copy(w3_hbm, w3_ref, sems.at[SW3])
        cp_w2 = lambda: pltpu.make_async_copy(w2_hbm, w2_ref, sems.at[SW2])

        def cp_x(blk):
            if isinstance(blk, int):
                src = x_hbm.at[blk * tm:(blk + 1) * tm, :]
            else:
                src = x_hbm.at[pl.ds(pl.multiple_of(blk * tm, tm), tm), :]
            return pltpu.make_async_copy(src, x_ref.at[blk], sems.at[SX + blk])

        def ln(dst_blk, src_blk, also=None, rows=8, chains=1):
            deps = [None] * chains
            t = 0
            for r0 in range(0, tm, 16):
                if rows == 8:
                    parts = []
                    for rr in (r0, r0 + 8):
                        y, deps[t % chains] = ln_f32(x_ref[src_blk, rr:rr + 8, :], deps[t % chains])
                        t += 1
                        parts.append(y)
                    xn = jnp.concatenate(parts, axis=0).astype(jnp.bfloat16)
                else:
                    y, deps[t % chains] = ln_f32(x_ref[src_blk, r0:r0 + 16, :], deps[t % chains])
                    t += 1
                    xn = y.astype(jnp.bfloat16)
                for kb in range(NB):
                    v = pack(xn[:, kb * 128:(kb + 1) * 128])
                    xn_ref[dst_blk, kb, r0 // 2:r0 // 2 + 8, :] = v
                    if also is not None:
                        also[kb, r0 // 2:r0 // 2 + 8, :] = v

        def ln_f32(x, dep):
            x = x.astype(jnp.float32)
            sm = jnp.sum(x, axis=-1, keepdims=True)
            if dep is not None:
                sm = sm + dep
            mu = sm * (1.0 / D)
            xc = x - mu
            var = jnp.mean(xc * xc, axis=-1, keepdims=True)
            rstd = lax.rsqrt(var + 1e-5)
            return xc * rstd, zero_dep(rstd)

        def load_act(get):
            return jnp.concatenate([unpack(get(kb)) for kb in range(NB)], axis=1)

        def proj(sec, off, lhs_ref, wblock):
            for j in range(NB):
                qkv_ref[sec, j, pl.ds(off, tm), :] = lax.dot_general(
                    load_act(lambda kb: lhs_ref[kb]), wblock(j), NT, preferred_element_type=jnp.float32)

        def wt_block(cb):
            return load_act(lambda kb: wt_ref[kb, cb * 64:(cb + 1) * 64, :])

        def wc_block(j):
            return load_act(lambda kb: wc_ref[kb, j * 64:(j + 1) * 64, :])

        def prep_wo_cols(j0, ncols):
            dep = None
            for jj in range(ncols):
                c0 = pl.multiple_of((j0 + jj) * 128, 128)
                for h in range(H):
                    blk = wo_ref[h * DH:(h + 1) * DH, pl.ds(c0, 128)].astype(jnp.float32)
                    if dep is not None:
                        blk = blk + dep
                    dep = zero_dep(blk[0:1, :])
                    t2_ref[jj, h * PS:h * PS + DH, :] = blk
                for d in range(DH):
                    blk = t2_ref[jj, pl.ds(d, H, stride=PS), :]
                    blk = blk + dep
                    dep = zero_dep(blk[0:1, :])
                    wop_ref[j0 + jj, d * (H // 2):(d + 1) * (H // 2), :] = pack(blk.astype(jnp.bfloat16))

        @pl.when(s == 0)
        def _prologue():
            for cp in (cp_x(0), cp_qa(), cp_qb(), cp_x(1), cp_sec(1), cp_x(2), cp_sec(2), cp_wo(), cp_x(3),
                       cp_w1(), cp_x(4), cp_w3(), cp_x(5), cp_x(6), cp_w2(), cp_x(7)):
                cp.start()
            qkv_ref[1:3, :, 0:HALO, :] = jnp.zeros((2, NB, HALO, 128), jnp.float32)
            eye = (lax.broadcasted_iota(jnp.int32, (128, 128), 0)
                   == lax.broadcasted_iota(jnp.int32, (128, 128), 1)).astype(jnp.bfloat16)

            def stage1(sec, cbs, xlu):
                dep = None
                for cb in cbs:
                    c0 = sec * D + cb * 128
                    w = wqkv_ref[:, c0:c0 + 128] if isinstance(c0, int) else wqkv_ref[:, pl.ds(pl.multiple_of(c0, 128), 128)]
                    if cb in xlu:
                        wf = w.astype(jnp.float32)
                        if dep is not None:
                            wf = wf + dep
                        tt = wf.T
                        if x_chain:
                            dep = zero_dep(tt[0:1, 0:128])
                    else:
                        tt = lax.dot_general(eye, w, NT, preferred_element_type=jnp.float32)
                    for hl in range(4):
                        r0 = (cb * 4 + hl) * PS
                        for kb in range(NB):
                            t_ref[kb, r0:r0 + DH, :] = tt[hl * DH:(hl + 1) * DH, kb * 128:(kb + 1) * 128]

            def stage2(sec):
                for d in range(DH):
                    r0 = d * (H // 2)
                    rd = pl.multiple_of(sec * (D // 2) + r0, H // 2)
                    for kb in range(NB):
                        blk = pack(t_ref[kb, pl.ds(d, H, stride=PS), :].astype(jnp.bfloat16))
                        wc_ref[kb, r0:r0 + H // 2, :] = blk
                        wt_ref[kb, pl.ds(rd, H // 2), :] = blk

            with scope("p_ln0"):
                cp_x(0).wait()

                def body(t, _):
                    for u in range(4):
                        r0 = pl.multiple_of(t * 64 + u * 16, 16)
                        rp = pl.multiple_of(t * 32 + u * 8, 8)
                        xn, _ = layernorm_bf16(x_ref[0, pl.ds(r0, 16), :])
                        for kb in range(NB):
                            v = pack(xn[:, kb * 128:(kb + 1) * 128])
                            xn_ref[0, kb, pl.ds(rp, 8), :] = v
                            xa_ref[kb, pl.ds(rp, 8), :] = v
                    return 0
                lax.fori_loop(0, tm // 64, body, 0)

            with scope("p_x0a"):
                cp_qa().wait()
                stage1(0, range(0, 4), xlu_blocks)
            with scope("p_x0b"):
                cp_qb().wait()
                stage1(0, range(4, 8), tuple(4 + c for c in xlu_blocks if c < 4))

            def sec_body(sec, _):
                @pl.when(sec == 0)
                def _():
                    cp_x(1).wait()
                stage2(sec)
                proj(sec, HALO, xa_ref, wc_block)
                ln(1, 1, also=xa1_ref, rows=p_rows, chains=p_chains)

                @pl.when(sec < 2)
                def _():
                    cp_sec(sec + 1).wait()

                @pl.when(sec == 0)
                def _():
                    cp_x(2).wait()
                proj(sec, HALO + tm, xa1_ref, wc_block)
                stage1(jnp.minimum(sec + 1, 2), range(NB), xlu2)
                ln(2, 2, rows=p_rows, chains=p_chains)
                return 0

            with scope("p_sec"):
                lax.fori_loop(0, 3, sec_body, 0)

        @pl.when(jnp.logical_and(s > 0, s < nblk - 1))
        def _seg_a():
          with scope("segA"):
            a = s + 1

            @pl.when(a < nblk - 1)
            def _():
                cp_x(a + 1).wait()

            @pl.when(s == 1)
            def _():
                cp_wo().wait()
            row0 = pl.multiple_of(a * tm, tm)
            for kb in range(NB):
                xa_ref[kb] = xn_ref[a, kb]
            for sec in range(3):
                proj(sec, HALO + row0, xa_ref, lambda j, sec=sec: wt_block(sec * NB + j))
            ln(a + 1, jnp.minimum(a + 1, nblk - 1))
            prep_wo_cols(jnp.minimum((s - 1) * 3, NB - 3), 3)

        @pl.when(s >= skew)
        def _seg_bc():
          with scope("segBC"):
            b = s - skew
            row0 = pl.multiple_of(b * tm, tm)

            @pl.when(s == skew)
            def _():
                cp_w1().wait()
                cp_w3().wait()
                cp_w2().wait()

            def load_xn():
                return load_act(lambda kb: xn_ref[b, kb])

            def ffn_chunk(c, acc):
                sl = slice(c * fc, (c + 1) * fc)
                g = jnp.dot(load_xn(), w1_ref[:, sl], preferred_element_type=jnp.float32)
                u = jnp.dot(load_xn(), w3_ref[:, sl], preferred_element_type=jnp.float32)
                h = (silu(g) * u).astype(jnp.bfloat16)
                t = jnp.dot(h, w2_ref[sl, :], preferred_element_type=jnp.float32)
                return t if acc is None else acc + t

            def attention():
                scale = DH ** -0.5
                a_rows = []
                dep = None
                for r in range(tm // ar):
                    r0 = r * ar
                    qs = [qkv_ref[0, j, pl.ds(row0 + (HALO + r0), ar), :] for j in range(NB)]
                    if dep is not None:
                        qs[0] = qs[0] + dep
                    logits = []
                    for w in range(W):
                        base = row0 + (HALO + r0 - DIL * w)
                        sc = qs[0] * qkv_ref[1, 0, pl.ds(base, ar), :]
                        for j in range(1, NB):
                            sc = sc + qs[j] * qkv_ref[1, j, pl.ds(base, ar), :]
                        sc = sc + pltpu.roll(sc, 64, 1)
                        sc = sc + pltpu.roll(sc, 32, 1)
                        sc = sc * scale
                        if r0 < DIL * w:
                            pos = row0 + r0 + lax.broadcasted_iota(jnp.int32, (ar, 128), 0)
                            sc = jnp.where(pos >= DIL * w, sc, -1e9)
                        logits.append(sc)
                    m = logits[0]
                    for w in range(1, W):
                        m = jnp.maximum(m, logits[w])
                    es = [jnp.exp(l - m) for l in logits]
                    den = es[0]
                    for w in range(1, W):
                        den = den + es[w]
                    inv = 1.0 / den
                    ps = [e * inv for e in es]
                    outs = []
                    for j in range(NB):
                        acc_a = None
                        for w in range(W):
                            base = row0 + (HALO + r0 - DIL * w)
                            t = ps[w] * qkv_ref[2, j, pl.ds(base, ar), :]
                            acc_a = t if acc_a is None else acc_a + t
                        outs.append(acc_a)
                    dep = zero_dep(outs[-1])
                    a_rows.append(jnp.concatenate(outs, axis=1))
                return jnp.concatenate(a_rows, axis=0).astype(jnp.bfloat16)

            def wo_matmul(a):
                wop = jnp.concatenate([unpack(wop_ref[j]) for j in range(NB)], axis=1)
                return jnp.dot(a, wop, preferred_element_type=jnp.float32)

            acc = None
            a = None
            s_out = None
            for c in range(nch):
                if c == attn_pos:
                    a = attention()
                if c == wo_pos:
                    s_out = wo_matmul(a)
                acc = ffn_chunk(c, acc)
            if wo_pos >= nch:
                s_out = wo_matmul(a)
            o_ref[...] = (x_ref[b].astype(jnp.float32) + s_out * silu(acc)).astype(o_ref.dtype)

    def fn(A_x, A_wqkv, A_wo, B_x, B_w1, B_w3, B_w2):
        x = A_x.reshape(S, D)
        anyspec = pl.BlockSpec(memory_space=pl.ANY)
        out = pl.pallas_call(
            kernel,
            grid=(nblk + skew,),
            in_specs=[anyspec] * 6,
            out_specs=pl.BlockSpec((tm, D), lambda s: (jnp.maximum(s - skew, 0), 0)),
            out_shape=jax.ShapeDtypeStruct((S, D), jnp.bfloat16),
            scratch_shapes=[
                pltpu.VMEM((D, 3 * D), jnp.bfloat16),
                pltpu.VMEM((D, D), jnp.bfloat16),
                pltpu.VMEM((D, F), jnp.bfloat16),
                pltpu.VMEM((D, F), jnp.bfloat16),
                pltpu.VMEM((F, D), jnp.bfloat16),
                pltpu.VMEM((NB, 3 * D // 2, 128), jnp.uint32),
                pltpu.VMEM((NB, D // 2, 128), jnp.uint32),
                pltpu.VMEM((NB, D // 2, 128), jnp.uint32),
                pltpu.VMEM((NB, H * PS, 128), jnp.float32),
                pltpu.VMEM((3, H * PS, 128), jnp.float32),
                pltpu.VMEM((nblk, tm, D), jnp.bfloat16),
                pltpu.VMEM((nblk + 1, NB, tm // 2, 128), jnp.uint32),
                pltpu.VMEM((NB, tm // 2, 128), jnp.uint32),
                pltpu.VMEM((NB, tm // 2, 128), jnp.uint32),
                pltpu.VMEM((3, NB, S + HALO, 128), jnp.float32),
                pltpu.SemaphoreType.DMA((SX + nblk,)),
            ],
            compiler_params=pltpu.CompilerParams(
                dimension_semantics=("arbitrary",), vmem_limit_bytes=120 * 1024 * 1024),
        )(x, A_wqkv, A_wo, B_w1, B_w3, B_w2)
        return out.reshape(1, S, D)

    return fn


_fn = _make_kernel()


@jax.jit
def pallas_recurrent_scan__sliding_local_dilated__glu_gated_swiglu__prompt_kernel(
    A_x: jax.Array,
    A_wqkv: jax.Array,
    A_wo: jax.Array,
    B_x: jax.Array,
    B_w1: jax.Array,
    B_w3: jax.Array,
    B_w2: jax.Array,
):
    return _fn(A_x, A_wqkv, A_wo, B_x, B_w1, B_w3, B_w2)
```

```python
import contextlib
import jax
import jax.numpy as jnp
from jax import lax
import jax.experimental.pallas as pl
import jax.experimental.pallas.tpu as pltpu

S, D, H, DH, F, W, DIL = 2048, 1024, 32, 32, 3584, 8, 2
HALO = 16
PS = 33
NT = (((1,), (1,)), ((), ()))
NB = D // 128


def zero_dep(x):
    return jnp.where(x > jnp.inf, 1.0, 0.0).astype(jnp.float32)


def silu(g):
    t = 0.5 * g
    return t + t * jnp.tanh(t)


def layernorm_bf16(x, dep=None):
    x = x.astype(jnp.float32)
    sm = jnp.sum(x, axis=-1, keepdims=True)
    if dep is not None:
        sm = sm + dep
    mu = sm * (1.0 / D)
    xc = x - mu
    var = jnp.mean(xc * xc, axis=-1, keepdims=True)
    rstd = lax.rsqrt(var + 1e-5)
    return (xc * rstd).astype(jnp.bfloat16), zero_dep(rstd)


def pack(x):
    return pltpu.bitcast(x, jnp.uint32)


def unpack(x):
    return pltpu.bitcast(x, jnp.bfloat16)


def _make_kernel(tm=256, fc=512, ar=8, skew=3, attn_pos=1, wo_pos=7, scopes=False, lr=8,
                xlu_blocks=(0, 1), x_chain=False, p_rows=8, p_chains=3, xlu2=(0, 1, 2, 3, 4, 5, 6, 7), osplit=4, a_rows=8, a_chains=1, wo_n=3):
    nblk = S // tm
    nch = F // fc
    scope = jax.named_scope if scopes else (lambda n: contextlib.nullcontext())
    SQB, SWO, SW1, SW3, SW2, SX = 3, 4, 5, 6, 7, 8

    def kernel(x_hbm, wqkv_hbm, wo_hbm, w1_hbm, w3_hbm, w2_hbm, o_hbm,
               wqkv_ref, wo_ref, w1_ref, w3_ref, w2_ref,
               wt_ref, wop_ref, wc_ref, t_ref, t2_ref, x_ref, xn_ref, xa_ref, qkv_ref, o_ref, sems, osems):
        s = pl.program_id(0)

        def cp_cols(c0, n, sem):
            sl = slice(c0, c0 + n) if isinstance(c0, int) else pl.ds(pl.multiple_of(c0, D), n)
            return pltpu.make_async_copy(wqkv_hbm.at[:, sl], wqkv_ref.at[:, sl], sems.at[sem])

        cp_qa = lambda: cp_cols(0, D // 2, 0)
        cp_qb = lambda: cp_cols(D // 2, D // 2, SQB)
        cp_sec = lambda sec: cp_cols(sec * D, D, sec)
        cp_wo = lambda: pltpu.make_async_copy(wo_hbm, wo_ref, sems.at[SWO])
        cp_w1 = lambda: pltpu.make_async_copy(w1_hbm, w1_ref, sems.at[SW1])
        cp_w3 = lambda: pltpu.make_async_copy(w3_hbm, w3_ref, sems.at[SW3])
        cp_w2 = lambda: pltpu.make_async_copy(w2_hbm, w2_ref, sems.at[SW2])

        def cp_x(blk):
            if isinstance(blk, int):
                src = x_hbm.at[blk * tm:(blk + 1) * tm, :]
            else:
                src = x_hbm.at[pl.ds(pl.multiple_of(blk * tm, tm), tm), :]
            return pltpu.make_async_copy(src, x_ref.at[blk], sems.at[SX + blk])

        def cp_out(blk, slot, p):
            cw = D // osplit
            cs = slice(p * cw, (p + 1) * cw)
            return pltpu.make_async_copy(o_ref.at[slot, :, cs],
                                         o_hbm.at[pl.ds(pl.multiple_of(blk * tm, tm), tm), cs],
                                         osems.at[slot * osplit + p])

        def ln(dst_blk, src_blk, also=None, rows=8, chains=1):
            deps = [None] * chains
            t = 0
            for r0 in range(0, tm, 16):
                if rows == 8:
                    parts = []
                    for rr in (r0, r0 + 8):
                        y, deps[t % chains] = ln_f32(x_ref[src_blk, rr:rr + 8, :], deps[t % chains])
                        t += 1
                        parts.append(y)
                    xn = jnp.concatenate(parts, axis=0).astype(jnp.bfloat16)
                else:
                    y, deps[t % chains] = ln_f32(x_ref[src_blk, r0:r0 + 16, :], deps[t % chains])
                    t += 1
                    xn = y.astype(jnp.bfloat16)
                for kb in range(NB):
                    v = pack(xn[:, kb * 128:(kb + 1) * 128])
                    xn_ref[dst_blk, kb, r0 // 2:r0 // 2 + 8, :] = v
                    if also is not None:
                        also[kb, r0 // 2:r0 // 2 + 8, :] = v

        def ln_f32(x, dep):
            x = x.astype(jnp.float32)
            sm = jnp.sum(x, axis=-1, keepdims=True)
            if dep is not None:
                sm = sm + dep
            mu = sm * (1.0 / D)
            xc = x - mu
            var = jnp.mean(xc * xc, axis=-1, keepdims=True)
            rstd = lax.rsqrt(var + 1e-5)
            return xc * rstd, zero_dep(rstd)

        def load_act(get):
            return jnp.concatenate([unpack(get(kb)) for kb in range(NB)], axis=1)

        def proj(sec, off, lhs, wblock):
            for j in range(NB):
                qkv_ref[sec, j, pl.ds(off, tm), :] = lax.dot_general(
                    load_act(lhs), wblock(j), NT, preferred_element_type=jnp.float32)

        def wt_block(cb):
            return load_act(lambda kb: wt_ref[kb, cb * 64:(cb + 1) * 64, :])

        def wc_block(j):
            return load_act(lambda kb: wc_ref[kb, j * 64:(j + 1) * 64, :])

        def prep_wo_cols(j0, ncols):
            dep = None
            for jj in range(ncols):
                c0 = pl.multiple_of((j0 + jj) * 128, 128)
                for h in range(H):
                    blk = wo_ref[h * DH:(h + 1) * DH, pl.ds(c0, 128)].astype(jnp.float32)
                    if dep is not None:
                        blk = blk + dep
                    dep = zero_dep(blk[0:1, :])
                    t2_ref[jj, h * PS:h * PS + DH, :] = blk
                for d in range(DH):
                    blk = t2_ref[jj, pl.ds(d, H, stride=PS), :]
                    blk = blk + dep
                    dep = zero_dep(blk[0:1, :])
                    wop_ref[j0 + jj, d * (H // 2):(d + 1) * (H // 2), :] = pack(blk.astype(jnp.bfloat16))

        @pl.when(s == 0)
        def _prologue():
            for cp in (cp_x(0), cp_qa(), cp_qb(), cp_x(1), cp_sec(1), cp_x(2), cp_sec(2), cp_wo(), cp_x(3),
                       cp_w1(), cp_x(4), cp_w3(), cp_x(5), cp_x(6), cp_w2(), cp_x(7)):
                cp.start()
            qkv_ref[1:3, :, 0:HALO, :] = jnp.zeros((2, NB, HALO, 128), jnp.float32)
            eye = (lax.broadcasted_iota(jnp.int32, (128, 128), 0)
                   == lax.broadcasted_iota(jnp.int32, (128, 128), 1)).astype(jnp.bfloat16)

            def stage1(sec, cbs, xlu):
                dep = None
                for cb in cbs:
                    c0 = sec * D + cb * 128
                    w = wqkv_ref[:, c0:c0 + 128] if isinstance(c0, int) else wqkv_ref[:, pl.ds(pl.multiple_of(c0, 128), 128)]
                    if cb in xlu:
                        wf = w.astype(jnp.float32)
                        if dep is not None:
                            wf = wf + dep
                        tt = wf.T
                        if x_chain:
                            dep = zero_dep(tt[0:1, 0:128])
                    else:
                        tt = lax.dot_general(eye, w, NT, preferred_element_type=jnp.float32)
                    for hl in range(4):
                        r0 = (cb * 4 + hl) * PS
                        for kb in range(NB):
                            t_ref[kb, r0:r0 + DH, :] = tt[hl * DH:(hl + 1) * DH, kb * 128:(kb + 1) * 128]

            def stage2(sec):
                for d in range(DH):
                    r0 = d * (H // 2)
                    rd = pl.multiple_of(sec * (D // 2) + r0, H // 2)
                    for kb in range(NB):
                        blk = pack(t_ref[kb, pl.ds(d, H, stride=PS), :].astype(jnp.bfloat16))
                        wc_ref[kb, r0:r0 + H // 2, :] = blk
                        wt_ref[kb, pl.ds(rd, H // 2), :] = blk

            with scope("p_ln0"):
                cp_x(0).wait()

                def body(t, _):
                    for u in range(4):
                        r0 = pl.multiple_of(t * 64 + u * 16, 16)
                        rp = pl.multiple_of(t * 32 + u * 8, 8)
                        xn, _ = layernorm_bf16(x_ref[0, pl.ds(r0, 16), :])
                        for kb in range(NB):
                            v = pack(xn[:, kb * 128:(kb + 1) * 128])
                            xn_ref[0, kb, pl.ds(rp, 8), :] = v
                            xa_ref[kb, pl.ds(rp, 8), :] = v
                    return 0
                lax.fori_loop(0, tm // 64, body, 0)

            with scope("p_x0a"):
                cp_qa().wait()
                stage1(0, range(0, 4), xlu_blocks)
            with scope("p_x0b"):
                cp_qb().wait()
                stage1(0, range(4, 8), tuple(4 + c for c in xlu_blocks if c < 4))

            def sec_body(sec, _):
                @pl.when(sec < 2)
                def _():
                    cp_x(sec + 1).wait()
                stage2(sec)
                proj(sec, HALO, lambda kb: xa_ref[kb], wc_block)
                lb = jnp.minimum(sec + 1, 2)
                ln(lb, lb, rows=p_rows, chains=p_chains)

                @pl.when(sec < 2)
                def _():
                    cp_sec(sec + 1).wait()
                proj(sec, HALO + tm, lambda kb: xn_ref[1, kb], wc_block)
                stage1(jnp.minimum(sec + 1, 2), range(NB), xlu2)
                return 0

            with scope("p_sec"):
                lax.fori_loop(0, 3, sec_body, 0)

        @pl.when(jnp.logical_and(s > 0, s < nblk - 1))
        def _seg_a():
          with scope("segA"):
            a = s + 1

            @pl.when(a < nblk - 1)
            def _():
                cp_x(a + 1).wait()

            @pl.when(s == 1)
            def _():
                cp_wo().wait()
            row0 = pl.multiple_of(a * tm, tm)
            for kb in range(NB):
                xa_ref[kb] = xn_ref[a, kb]
            for sec in range(3):
                proj(sec, HALO + row0, lambda kb: xa_ref[kb], lambda j, sec=sec: wt_block(sec * NB + j))
            ln(a + 1, jnp.minimum(a + 1, nblk - 1), rows=a_rows, chains=a_chains)
            prep_wo_cols(jnp.minimum((s - 1) * wo_n, NB - wo_n), wo_n)

        @pl.when(s >= skew)
        def _seg_bc():
          with scope("segBC"):
            b = s - skew
            row0 = pl.multiple_of(b * tm, tm)

            @pl.when(s == skew)
            def _():
                cp_w1().wait()
                cp_w3().wait()
                cp_w2().wait()

            @pl.when(b >= 2)
            def _():
                for p in range(osplit):
                    cp_out(b - 2, b % 2, p).wait()

            def load_xn():
                return load_act(lambda kb: xn_ref[b, kb])

            def ffn_chunk(c, acc):
                sl = slice(c * fc, (c + 1) * fc)
                g = jnp.dot(load_xn(), w1_ref[:, sl], preferred_element_type=jnp.float32)
                u = jnp.dot(load_xn(), w3_ref[:, sl], preferred_element_type=jnp.float32)
                h = (silu(g) * u).astype(jnp.bfloat16)
                t = jnp.dot(h, w2_ref[sl, :], preferred_element_type=jnp.float32)
                return t if acc is None else acc + t

            def attention():
                scale = DH ** -0.5
                a_rows = []
                dep = None
                for r in range(tm // ar):
                    r0 = r * ar
                    qs = [qkv_ref[0, j, pl.ds(row0 + (HALO + r0), ar), :] for j in range(NB)]
                    if dep is not None:
                        qs[0] = qs[0] + dep
                    logits = []
                    for w in range(W):
                        base = row0 + (HALO + r0 - DIL * w)
                        sc = qs[0] * qkv_ref[1, 0, pl.ds(base, ar), :]
                        for j in range(1, NB):
                            sc = sc + qs[j] * qkv_ref[1, j, pl.ds(base, ar), :]
                        sc = sc + pltpu.roll(sc, 64, 1)
                        sc = sc + pltpu.roll(sc, 32, 1)
                        sc = sc * scale
                        if r0 < DIL * w:
                            pos = row0 + r0 + lax.broadcasted_iota(jnp.int32, (ar, 128), 0)
                            sc = jnp.where(pos >= DIL * w, sc, -1e9)
                        logits.append(sc)
                    m = logits[0]
                    for w in range(1, W):
                        m = jnp.maximum(m, logits[w])
                    es = [jnp.exp(l - m) for l in logits]
                    den = es[0]
                    for w in range(1, W):
                        den = den + es[w]
                    inv = 1.0 / den
                    ps = [e * inv for e in es]
                    outs = []
                    for j in range(NB):
                        acc_a = None
                        for w in range(W):
                            base = row0 + (HALO + r0 - DIL * w)
                            t = ps[w] * qkv_ref[2, j, pl.ds(base, ar), :]
                            acc_a = t if acc_a is None else acc_a + t
                        outs.append(acc_a)
                    dep = zero_dep(outs[-1])
                    a_rows.append(jnp.concatenate(outs, axis=1))
                return jnp.concatenate(a_rows, axis=0).astype(jnp.bfloat16)

            def wo_matmul(a):
                wop = jnp.concatenate([unpack(wop_ref[j]) for j in range(NB)], axis=1)
                return jnp.dot(a, wop, preferred_element_type=jnp.float32)

            acc = None
            a = None
            s_out = None
            for c in range(nch):
                if c == attn_pos:
                    a = attention()
                if c == wo_pos:
                    s_out = wo_matmul(a)
                acc = ffn_chunk(c, acc)
            if wo_pos >= nch:
                s_out = wo_matmul(a)
            slot = b % 2
            gg = silu(acc)
            cw = D // osplit
            for p in range(osplit):
                cs = slice(p * cw, (p + 1) * cw)
                o_ref[slot, :, cs] = (x_ref[b, :, cs].astype(jnp.float32) + s_out[:, cs] * gg[:, cs]).astype(o_ref.dtype)
                cp_out(b, slot, p).start()

            @pl.when(b == nblk - 1)
            def _():
                for p in range(osplit):
                    cp_out(b - 1, 1 - slot, p).wait()
                for p in range(osplit):
                    cp_out(b, slot, p).wait()

    def fn(A_x, A_wqkv, A_wo, B_x, B_w1, B_w3, B_w2):
        x = A_x.reshape(S, D)
        anyspec = pl.BlockSpec(memory_space=pl.ANY)
        out = pl.pallas_call(
            kernel,
            grid=(nblk + skew,),
            in_specs=[anyspec] * 6,
            out_specs=anyspec,
            out_shape=jax.ShapeDtypeStruct((S, D), jnp.bfloat16),
            scratch_shapes=[
                pltpu.VMEM((D, 3 * D), jnp.bfloat16),
                pltpu.VMEM((D, D), jnp.bfloat16),
                pltpu.VMEM((D, F), jnp.bfloat16),
                pltpu.VMEM((D, F), jnp.bfloat16),
                pltpu.VMEM((F, D), jnp.bfloat16),
                pltpu.VMEM((NB, 3 * D // 2, 128), jnp.uint32),
                pltpu.VMEM((NB, D // 2, 128), jnp.uint32),
                pltpu.VMEM((NB, D // 2, 128), jnp.uint32),
                pltpu.VMEM((NB, H * PS, 128), jnp.float32),
                pltpu.VMEM((wo_n, H * PS, 128), jnp.float32),
                pltpu.VMEM((nblk, tm, D), jnp.bfloat16),
                pltpu.VMEM((nblk + 1, NB, tm // 2, 128), jnp.uint32),
                pltpu.VMEM((NB, tm // 2, 128), jnp.uint32),
                pltpu.VMEM((3, NB, S + HALO, 128), jnp.float32),
                pltpu.VMEM((2, tm, D), jnp.bfloat16),
                pltpu.SemaphoreType.DMA((SX + nblk,)),
                pltpu.SemaphoreType.DMA((2 * osplit,)),
            ],
            compiler_params=pltpu.CompilerParams(
                dimension_semantics=("arbitrary",), vmem_limit_bytes=120 * 1024 * 1024),
        )(x, A_wqkv, A_wo, B_w1, B_w3, B_w2)
        return out.reshape(1, S, D)

    return fn


_fn = _make_kernel()


@jax.jit
def pallas_recurrent_scan__sliding_local_dilated__glu_gated_swiglu__prompt_kernel(
    A_x: jax.Array,
    A_wqkv: jax.Array,
    A_wo: jax.Array,
    B_x: jax.Array,
    B_w1: jax.Array,
    B_w3: jax.Array,
    B_w2: jax.Array,
):
    return _fn(A_x, A_wqkv, A_wo, B_x, B_w1, B_w3, B_w2)
```

```python
import jax
import jax.numpy as jnp
from jax import lax
import jax.experimental.pallas as pl
import jax.experimental.pallas.tpu as pltpu

S, D, H, DH, F, W, DIL = 2048, 1024, 32, 32, 3584, 8, 2
TM = 256
NBLK = S // TM
FC = 512
SKEW = 3
AR = 8
HALO = 16
PS = 33
NB = D // 128
OSPLIT = 4
WO_N = 3
NT = (((1,), (1,)), ((), ()))
SQB, SWO, SW1, SW3, SW2, SX = 3, 4, 5, 6, 7, 8


def _zero_dep(x):
    return jnp.where(x > jnp.inf, 1.0, 0.0).astype(jnp.float32)


def _silu(g):
    t = 0.5 * g
    return t + t * jnp.tanh(t)


def _layernorm(x, dep=None):
    x = x.astype(jnp.float32)
    sm = jnp.sum(x, axis=-1, keepdims=True)
    if dep is not None:
        sm = sm + dep
    mu = sm * (1.0 / D)
    xc = x - mu
    var = jnp.mean(xc * xc, axis=-1, keepdims=True)
    rstd = lax.rsqrt(var + 1e-5)
    return xc * rstd, _zero_dep(rstd)


def _pack(x):
    return pltpu.bitcast(x, jnp.uint32)


def _unpack(x):
    return pltpu.bitcast(x, jnp.bfloat16)


def _lanes(get):
    return jnp.concatenate([_unpack(get(kb)) for kb in range(NB)], axis=1)


def _kernel(x_hbm, wqkv_hbm, wo_hbm, w1_hbm, w3_hbm, w2_hbm, o_hbm,
            wqkv_ref, wo_ref, w1_ref, w3_ref, w2_ref,
            wt_ref, wop_ref, wc_ref, t_ref, t2_ref, x_ref, xn_ref, xa_ref, qkv_ref, o_ref, sems, osems):
    s = pl.program_id(0)

    def cp_cols(c0, n, sem):
        sl = slice(c0, c0 + n) if isinstance(c0, int) else pl.ds(pl.multiple_of(c0, D), n)
        return pltpu.make_async_copy(wqkv_hbm.at[:, sl], wqkv_ref.at[:, sl], sems.at[sem])

    cp_qa = lambda: cp_cols(0, D // 2, 0)
    cp_qb = lambda: cp_cols(D // 2, D // 2, SQB)
    cp_sec = lambda sec: cp_cols(sec * D, D, sec)
    cp_wo = lambda: pltpu.make_async_copy(wo_hbm, wo_ref, sems.at[SWO])
    cp_w1 = lambda: pltpu.make_async_copy(w1_hbm, w1_ref, sems.at[SW1])
    cp_w3 = lambda: pltpu.make_async_copy(w3_hbm, w3_ref, sems.at[SW3])
    cp_w2 = lambda: pltpu.make_async_copy(w2_hbm, w2_ref, sems.at[SW2])

    def rows_of(blk):
        if isinstance(blk, int):
            return slice(blk * TM, (blk + 1) * TM)
        return pl.ds(pl.multiple_of(blk * TM, TM), TM)

    def cp_x(blk):
        return pltpu.make_async_copy(x_hbm.at[rows_of(blk), :], x_ref.at[blk], sems.at[SX + blk])

    def cp_out(blk, slot, p):
        cs = slice(p * (D // OSPLIT), (p + 1) * (D // OSPLIT))
        return pltpu.make_async_copy(o_ref.at[slot, :, cs], o_hbm.at[rows_of(blk), cs], osems.at[slot])

    def wait_out(blk, slot):
        pltpu.make_async_copy(o_ref.at[slot], o_hbm.at[rows_of(blk), :], osems.at[slot]).wait()

    def layernorm_block(blk_dst, blk_src, chains):
        deps = [None] * chains
        t = 0
        for r0 in range(0, TM, 16):
            parts = []
            for rr in (r0, r0 + 8):
                y, deps[t % chains] = _layernorm(x_ref[blk_src, rr:rr + 8, :], deps[t % chains])
                t += 1
                parts.append(y)
            xn = jnp.concatenate(parts, axis=0).astype(jnp.bfloat16)
            for kb in range(NB):
                xn_ref[blk_dst, kb, r0 // 2:r0 // 2 + 8, :] = _pack(xn[:, kb * 128:(kb + 1) * 128])

    def project(sec, off, lhs, wblock):
        for j in range(NB):
            qkv_ref[sec, j, pl.ds(off, TM), :] = lax.dot_general(
                _lanes(lhs), wblock(j), NT, preferred_element_type=jnp.float32)

    def permute_wo_cols(j0):
        dep = None
        for jj in range(WO_N):
            c0 = pl.multiple_of((j0 + jj) * 128, 128)
            for h in range(H):
                blk = wo_ref[h * DH:(h + 1) * DH, pl.ds(c0, 128)].astype(jnp.float32)
                if dep is not None:
                    blk = blk + dep
                dep = _zero_dep(blk[0:1, :])
                t2_ref[jj, h * PS:h * PS + DH, :] = blk
            for d in range(DH):
                blk = t2_ref[jj, pl.ds(d, H, stride=PS), :] + dep
                dep = _zero_dep(blk[0:1, :])
                wop_ref[j0 + jj, d * (H // 2):(d + 1) * (H // 2), :] = _pack(blk.astype(jnp.bfloat16))

    @pl.when(s == 0)
    def _prologue():
        for cp in (cp_x(0), cp_qa(), cp_qb(), cp_x(1), cp_sec(1), cp_x(2), cp_sec(2), cp_wo(), cp_x(3),
                   cp_w1(), cp_x(4), cp_w3(), cp_x(5), cp_x(6), cp_w2(), cp_x(7)):
            cp.start()
        qkv_ref[1:3, :, 0:HALO, :] = jnp.zeros((2, NB, HALO, 128), jnp.float32)
        eye = (lax.broadcasted_iota(jnp.int32, (128, 128), 0)
               == lax.broadcasted_iota(jnp.int32, (128, 128), 1)).astype(jnp.bfloat16)

        def transpose_cols(sec, cbs, on_xlu):
            for cb in cbs:
                c0 = sec * D + cb * 128
                if isinstance(c0, int):
                    w = wqkv_ref[:, c0:c0 + 128]
                else:
                    w = wqkv_ref[:, pl.ds(pl.multiple_of(c0, 128), 128)]
                if cb in on_xlu:
                    tt = w.astype(jnp.float32).T
                else:
                    tt = lax.dot_general(eye, w, NT, preferred_element_type=jnp.float32)
                for hl in range(4):
                    r0 = (cb * 4 + hl) * PS
                    for kb in range(NB):
                        t_ref[kb, r0:r0 + DH, :] = tt[hl * DH:(hl + 1) * DH, kb * 128:(kb + 1) * 128]

        def gather_rows(sec):
            for d in range(DH):
                r0 = d * (H // 2)
                rd = pl.multiple_of(sec * (D // 2) + r0, H // 2)
                for kb in range(NB):
                    blk = _pack(t_ref[kb, pl.ds(d, H, stride=PS), :].astype(jnp.bfloat16))
                    wc_ref[kb, r0:r0 + H // 2, :] = blk
                    wt_ref[kb, pl.ds(rd, H // 2), :] = blk

        cp_x(0).wait()

        def ln0_body(t, _):
            for u in range(4):
                r0 = pl.multiple_of(t * 64 + u * 16, 16)
                rp = pl.multiple_of(t * 32 + u * 8, 8)
                y, _unused = _layernorm(x_ref[0, pl.ds(r0, 16), :])
                xn = y.astype(jnp.bfloat16)
                for kb in range(NB):
                    v = _pack(xn[:, kb * 128:(kb + 1) * 128])
                    xn_ref[0, kb, pl.ds(rp, 8), :] = v
                    xa_ref[kb, pl.ds(rp, 8), :] = v
            return 0
        lax.fori_loop(0, TM // 64, ln0_body, 0)

        cp_qa().wait()
        transpose_cols(0, range(0, 4), (0, 1))
        cp_qb().wait()
        transpose_cols(0, range(4, 8), (4, 5))

        wc_block = lambda j: _lanes(lambda kb: wc_ref[kb, j * 64:(j + 1) * 64, :])

        def sec_body(sec, _):
            @pl.when(sec < 2)
            def _():
                cp_x(sec + 1).wait()
            gather_rows(sec)
            project(sec, HALO, lambda kb: xa_ref[kb], wc_block)
            lb = jnp.minimum(sec + 1, 2)
            layernorm_block(lb, lb, chains=3)

            @pl.when(sec < 2)
            def _():
                cp_sec(sec + 1).wait()
            project(sec, HALO + TM, lambda kb: xn_ref[1, kb], wc_block)
            transpose_cols(jnp.minimum(sec + 1, 2), range(NB), range(NB))
            return 0

        lax.fori_loop(0, 3, sec_body, 0)

    @pl.when(jnp.logical_and(s > 0, s < NBLK - 1))
    def _seg_a():
        a = s + 1

        @pl.when(a < NBLK - 1)
        def _():
            cp_x(a + 1).wait()

        @pl.when(s == 1)
        def _():
            cp_wo().wait()
        row0 = pl.multiple_of(a * TM, TM)
        for kb in range(NB):
            xa_ref[kb] = xn_ref[a, kb]
        for sec in range(3):
            project(sec, HALO + row0, lambda kb: xa_ref[kb],
                    lambda j, sec=sec: _lanes(
                        lambda kb: wt_ref[kb, (sec * NB + j) * 64:(sec * NB + j + 1) * 64, :]))
        layernorm_block(a + 1, jnp.minimum(a + 1, NBLK - 1), chains=1)
        permute_wo_cols(jnp.minimum((s - 1) * WO_N, NB - WO_N))

    @pl.when(s >= SKEW)
    def _seg_bc():
        b = s - SKEW
        row0 = pl.multiple_of(b * TM, TM)

        @pl.when(s == SKEW)
        def _():
            cp_w1().wait()
            cp_w3().wait()
            cp_w2().wait()

        @pl.when(b >= 2)
        def _():
            wait_out(b - 2, b & 1)

        def ffn_chunk(c, acc):
            sl = slice(c * FC, (c + 1) * FC)
            g = jnp.dot(_lanes(lambda kb: xn_ref[b, kb]), w1_ref[:, sl], preferred_element_type=jnp.float32)
            u = jnp.dot(_lanes(lambda kb: xn_ref[b, kb]), w3_ref[:, sl], preferred_element_type=jnp.float32)
            h = (_silu(g) * u).astype(jnp.bfloat16)
            t = jnp.dot(h, w2_ref[sl, :], preferred_element_type=jnp.float32)
            return t if acc is None else acc + t

        def attention():
            scale = DH ** -0.5
            a_rows = []
            dep = None
            for r0 in range(0, TM, AR):
                qs = [qkv_ref[0, j, pl.ds(row0 + (HALO + r0), AR), :] for j in range(NB)]
                if dep is not None:
                    qs[0] = qs[0] + dep
                logits = []
                for w in range(W):
                    base = row0 + (HALO + r0 - DIL * w)
                    sc = qs[0] * qkv_ref[1, 0, pl.ds(base, AR), :]
                    for j in range(1, NB):
                        sc = sc + qs[j] * qkv_ref[1, j, pl.ds(base, AR), :]
                    sc = sc + pltpu.roll(sc, 64, 1)
                    sc = sc + pltpu.roll(sc, 32, 1)
                    sc = sc * scale
                    if r0 < DIL * w:
                        pos = row0 + r0 + lax.broadcasted_iota(jnp.int32, (AR, 128), 0)
                        sc = jnp.where(pos >= DIL * w, sc, -1e9)
                    logits.append(sc)
                m = logits[0]
                for w in range(1, W):
                    m = jnp.maximum(m, logits[w])
                es = [jnp.exp(l - m) for l in logits]
                den = es[0]
                for w in range(1, W):
                    den = den + es[w]
                inv = 1.0 / den
                ps = [e * inv for e in es]
                outs = []
                for j in range(NB):
                    acc_a = None
                    for w in range(W):
                        base = row0 + (HALO + r0 - DIL * w)
                        t = ps[w] * qkv_ref[2, j, pl.ds(base, AR), :]
                        acc_a = t if acc_a is None else acc_a + t
                    outs.append(acc_a)
                dep = _zero_dep(outs[-1])
                a_rows.append(jnp.concatenate(outs, axis=1))
            return jnp.concatenate(a_rows, axis=0).astype(jnp.bfloat16)

        acc = ffn_chunk(0, None)
        att = attention()
        for c in range(1, F // FC):
            acc = ffn_chunk(c, acc)
        wop = jnp.concatenate([_unpack(wop_ref[j]) for j in range(NB)], axis=1)
        s_out = jnp.dot(att, wop, preferred_element_type=jnp.float32)
        gate = _silu(acc)
        slot = b & 1
        for p in range(OSPLIT):
            cs = slice(p * (D // OSPLIT), (p + 1) * (D // OSPLIT))
            o_ref[slot, :, cs] = (x_ref[b, :, cs].astype(jnp.float32)
                                  + s_out[:, cs] * gate[:, cs]).astype(o_ref.dtype)
            cp_out(b, slot, p).start()

        @pl.when(b == NBLK - 1)
        def _():
            wait_out(b - 1, 1 - slot)
            wait_out(b, slot)


@jax.jit
def pallas_recurrent_scan__sliding_local_dilated__glu_gated_swiglu__prompt_kernel(
    A_x: jax.Array,
    A_wqkv: jax.Array,
    A_wo: jax.Array,
    B_x: jax.Array,
    B_w1: jax.Array,
    B_w3: jax.Array,
    B_w2: jax.Array,
):
    x = A_x.reshape(S, D)
    out = pl.pallas_call(
        _kernel,
        grid=(NBLK + SKEW,),
        in_specs=[pl.BlockSpec(memory_space=pl.ANY)] * 6,
        out_specs=pl.BlockSpec(memory_space=pl.ANY),
        out_shape=jax.ShapeDtypeStruct((S, D), jnp.bfloat16),
        scratch_shapes=[
            pltpu.VMEM((D, 3 * D), jnp.bfloat16),
            pltpu.VMEM((D, D), jnp.bfloat16),
            pltpu.VMEM((D, F), jnp.bfloat16),
            pltpu.VMEM((D, F), jnp.bfloat16),
            pltpu.VMEM((F, D), jnp.bfloat16),
            pltpu.VMEM((NB, 3 * D // 2, 128), jnp.uint32),
            pltpu.VMEM((NB, D // 2, 128), jnp.uint32),
            pltpu.VMEM((NB, D // 2, 128), jnp.uint32),
            pltpu.VMEM((NB, H * PS, 128), jnp.float32),
            pltpu.VMEM((WO_N, H * PS, 128), jnp.float32),
            pltpu.VMEM((NBLK, TM, D), jnp.bfloat16),
            pltpu.VMEM((NBLK + 1, NB, TM // 2, 128), jnp.uint32),
            pltpu.VMEM((NB, TM // 2, 128), jnp.uint32),
            pltpu.VMEM((3, NB, S + HALO, 128), jnp.float32),
            pltpu.VMEM((2, TM, D), jnp.bfloat16),
            pltpu.SemaphoreType.DMA((SX + NBLK,)),
            pltpu.SemaphoreType.DMA((2,)),
        ],
        compiler_params=pltpu.CompilerParams(
            dimension_semantics=("arbitrary",), vmem_limit_bytes=120 * 1024 * 1024),
    )(x, A_wqkv, A_wo, B_w1, B_w3, B_w2)
    return out.reshape(1, S, D)
```
